```python
import jax
import jax.numpy as jnp

def _softmax(x, axis=-1):
    return jax.nn.softmax(x, axis=axis)
def _gelu(x):
    return jax.nn.gelu(x, approximate=True)
def _silu(x):
    return jax.nn.silu(x)
def _sigmoid(x):
    return jax.nn.sigmoid(x)
def _layernorm(x, axis=-1, eps=1e-5):
    m = jnp.mean(x, axis=axis, keepdims=True)
    v = jnp.var(x, axis=axis, keepdims=True)
    return (x - m) / jnp.sqrt(v + eps)
def _scatter_add(tgt, idx, src, axis=0):
    return tgt.at[idx].add(src)
def _segment_sum(src, seg, n):
    return jax.ops.segment_sum(src, seg, n)
class _Rng:
    def __init__(self, key):
        self._k = key
    def _next(self):
        self._k, sub = jax.random.split(self._k)
        return sub
    def normal(self, shape):
        return jax.random.normal(self._next(), shape, dtype=jnp.bfloat16)
    def randint(self, lo, hi, shape):
        return jax.random.randint(self._next(), shape, lo, hi, dtype=jnp.int32)
    def uniform(self, shape, lo=0.0, hi=1.0):
        return jax.random.uniform(self._next(), shape, jnp.bfloat16, lo, hi)
    def permutation(self, n):
        return jax.random.permutation(self._next(), n)


kernel_name = 'standalone__channel_attn_se__vision'

def _fwd_setup_inputs():
    _rng = _Rng(jax.random.key(int.from_bytes(__import__("os").urandom(4), "little")))
    _w = (lambda a: (lambda t: t.astype(jnp.bfloat16) if jnp.issubdtype(t.dtype, jnp.floating) else t)(jnp.asarray(a)))
    H = W = 384
    C = 96
    r = max(C // 16, 4)
    return {
        "x": _w((lambda *s: _rng.normal(s) * 0.05)(1, H, W, C)),
        "w_down": _w((lambda *s: _rng.normal(s) * 0.05)(C, r)),
        "w_up": _w((lambda *s: _rng.normal(s) * 0.05)(r, C)),
    }

def _fwd_reference(x, w_down, w_up):
    s = x.mean(axis=(1, 2))
    h = _silu(jnp.einsum('bc,cr->br', s, w_down))
    g = _sigmoid(jnp.einsum('br,rc->bc', h, w_up))
    return x * g[:, None, None, :]


def setup_inputs():
    _inp = _fwd_setup_inputs()
    _gk = jax.random.fold_in(jax.random.key(int.from_bytes(__import__("os").urandom(4), "little")), 2**31 - 1)
    _shapes = [[1, 384, 384, 96]]
    _dtypes = ['bfloat16']
    _gks = jax.random.split(_gk, len(_shapes))
    _gs = [jax.random.normal(k, s, dtype=jnp.dtype(d)) * 0.05 for k, s, d in zip(_gks, _shapes, _dtypes)]
    _inp["grad_out"] = _gs[0]
    return _inp

def reference(x, w_down, w_up, grad_out):
    _const = dict()
    def _f(*_d):
        return _fwd_reference(**{'x': _d[0], 'w_down': _d[1], 'w_up': _d[2], **_const})
    _out, _vjp = jax.vjp(_f, x, w_down, w_up)
    _grads = _vjp(grad_out)
    _out0 = jnp.asarray(_out)
    return (_out0, *[jnp.asarray(_g) for _g in _grads])
```

```python
import jax
import jax.numpy as jnp
from jax import lax
import jax.experimental.pallas as pl
import jax.experimental.pallas.tpu as pltpu

F32 = jnp.float32
BF16 = jnp.bfloat16

LANES = 128
SUBLANES = 8

BLOCK = 4096
READ_PIECE = 128
WRITE_PIECE = 80
WRITE_STREAMS = 7

SLOTS = 9
CYCLED = (400, 400) + (432,) * 9
PARKED = (448,) * SLOTS
FIRST_READS = 20
RING_STEPS = (
    ((1, 1, 0, 4), (3, 2, 1, 5), (5, 3, 2, 5), (7, 4, 3, 8), (9, 6, 4, 6), (9, 6, 5, 6)),
    ((9, 8, 6, 9),),
    ((9, 9, 7, 9), (10, 10, 8, 0), (11, 11, 11, 0)),
)

UNROLL = 2


@jax.jit
def pallas_standalone__channel_attn_se__vision_kernel(
    x: jax.Array,
    w_down: jax.Array,
    w_up: jax.Array,
    grad_out: jax.Array,
):
    batch, H, W, C = x.shape
    R = w_down.shape[1]
    assert batch == 1 and C % (2 * SUBLANES) == 0 and W % LANES == 0
    CT, WT = C // SUBLANES, W // LANES
    ROWS = CT * WT * SUBLANES
    GROUP = 2 * WT * SUBLANES
    NG = ROWS // GROUP
    assert (H * ROWS) % BLOCK == 0
    NB = H * ROWS // BLOCK
    inv_n = 1.0 / (H * W)

    sizes = CYCLED + PARKED
    n_cyc, n_chunks = len(CYCLED), len(CYCLED) + SLOTS
    where, main_end, blk = [], [BLOCK] * NB, NB - 1
    for size in reversed(sizes):
        blk -= main_end[blk] < size
        main_end[blk] -= size
        where.insert(0, (blk, main_end[blk]))
    assert main_end == sorted(main_end, reverse=True)
    assert RING_STEPS[-1][-1][:3] == (n_cyc,) * 3

    x_plan = [(NB, r, READ_PIECE) for r in range(0, BLOCK, READ_PIECE)]
    cuts = sorted({*range(0, BLOCK, READ_PIECE), *main_end})
    go_plan = [(sum(e >= hi for e in main_end), lo, hi - lo) for lo, hi in zip(cuts, cuts[1:])]

    groups = [(b, min(WRITE_STREAMS, NB - b)) for b in range(0, NB, WRITE_STREAMS)]
    columns = BLOCK // WRITE_PIECE
    assert len(groups) == 4 and WRITE_PIECE % (2 * SUBLANES) == 0

    early = (where[n_cyc][0] * BLOCK + where[n_cyc][1]) // ROWS // (2 * UNROLL) * (2 * UNROLL)

    def to_view(t):
        t = t.reshape(H, WT, LANES, CT, SUBLANES).transpose(0, 3, 1, 4, 2)
        return t.reshape(NB, BLOCK, LANES)

    def from_view(t):
        t = t.reshape(H, CT, WT, SUBLANES, LANES).transpose(0, 2, 4, 1, 3)
        return t.reshape(1, H, W, C)

    def load(ref, h, q):
        v = ref.reshape(H, ROWS, LANES)[h, q * GROUP:(q + 1) * GROUP, :]
        return v.astype(F32).reshape(2, WT, SUBLANES, LANES)

    def store(ref, h, q, v):
        v = v.reshape(GROUP, LANES).astype(BF16)
        ref.reshape(H, ROWS, LANES)[h, q * GROUP:(q + 1) * GROUP, :] = v

    def slab_loop(lo, hi, slab_step, init):
        assert lo % UNROLL == 0 and hi % UNROLL == 0

        def step(i, carry):
            for k in range(UNROLL):
                carry = slab_step(i * UNROLL + k, carry)
            return carry

        return lax.fori_loop(lo // UNROLL, hi // UNROLL, step, init)

    def fold(v):
        r = v[:, 0]
        for k in range(1, WT):
            r = r + v[:, k]
        return r

    def diag(v):
        eye = (lax.broadcasted_iota(jnp.int32, (C, C), 0)
               == lax.broadcasted_iota(jnp.int32, (C, C), 1))
        return jnp.where(eye, jnp.broadcast_to(v, (C, C)), 0.0)

    def acc_to_row(acc):
        a = jnp.concatenate(acc, axis=0).reshape(C, LANES)
        return jnp.sum(diag(jnp.sum(a, axis=1, keepdims=True)), axis=0, keepdims=True)

    def row_to_tiles(row):
        col = jnp.sum(diag(row), axis=1, keepdims=True)
        t = jnp.broadcast_to(col, (C, LANES)).reshape(NG, 2, 1, SUBLANES, LANES)
        return [t[q] for q in range(NG)]

    def body(x_hbm, wd_hbm, wu_hbm, go_hbm, o_hbm, gx_hbm, gwd_hbm, gwu_hbm,
             xb, gb, ob, wd_v, wu_v, gwd_v, gwu_v, ring,
             x_sem, go_sem, out_sem, gx_sem, w_sems, ring_sems):
        copy = pltpu.make_async_copy
        out_route, gx_route = (ob, o_hbm, out_sem), (xb, gx_hbm, gx_sem)

        def strided(src, dst, block, pieces, row, rows, sem):
            sl = (pl.ds(block, pieces), pl.ds(row, rows), slice(None))
            return copy(src.at[sl], dst.at[sl], sem)

        def start_writes(route, group, lo=0, hi=columns):
            src, dst, sem = route

            def step(j, carry):
                row = pl.multiple_of(j * WRITE_PIECE, 2 * SUBLANES)
                strided(src, dst, *group, row, WRITE_PIECE, sem).start()
                return carry

            lax.fori_loop(lo, min(hi, columns - 1), step, 0)
            if hi == columns:
                row = (columns - 1) * WRITE_PIECE
                strided(src, dst, *group, row, BLOCK - row, sem).start()

        def to_ring(u):
            b, r = where[u]
            return copy(go_hbm.at[b, pl.ds(r, sizes[u])],
                        ring.at[u % SLOTS, pl.ds(0, sizes[u])], ring_sems.at[u % SLOTS])

        def from_ring(u):
            b, r = where[u]
            return copy(ring.at[u % SLOTS, pl.ds(0, sizes[u])],
                        gb.at[b, pl.ds(r, sizes[u])], ring_sems.at[u % SLOTS])

        rd_x = [strided(x_hbm, xb, 0, *p, x_sem) for p in x_plan]
        rd_w = [copy(wd_hbm, wd_v, w_sems.at[0]), copy(wu_hbm, wu_v, w_sems.at[1])]
        rd_go = [strided(go_hbm, gb, 0, *p, go_sem) for p in go_plan]
        pending = rd_x[:1] + rd_w + rd_x[1:] + rd_go

        def feed(n):
            for c in pending[:n]:
                c.start()
            del pending[:n]

        done = [0, 0, 0]

        def ring_steps(steps):
            for filled, draining, drained, reads in steps:
                assert drained <= draining <= filled <= done[2] + SLOTS
                for u in range(done[0], filled):
                    to_ring(u).wait()
                for u in range(done[1], draining):
                    from_ring(u).start()
                for u in range(done[2], drained):
                    from_ring(u).wait()
                    to_ring(u + SLOTS).start()
                done[:] = filled, draining, drained
                feed(reads)

        feed(1)
        for u in range(SLOTS):
            to_ring(u).start()
        feed(FIRST_READS - 1)
        ring_steps(RING_STEPS[0])
        assert len(pending) <= len(rd_go)

        zeros = tuple(jnp.zeros((2, SUBLANES, LANES), F32) for _ in range(NG))

        def sum_step(h, acc):
            return tuple(acc[q] + fold(load(xb, h, q)) for q in range(NG))

        for c in rd_w + rd_x:
            c.wait()
        acc = slab_loop(0, H, sum_step, zeros)
        wd = wd_v[...].astype(F32)
        wu = wu_v[...].astype(F32)
        s = acc_to_row(acc) * inv_n
        z1 = jnp.sum(wd * s, axis=1, keepdims=True)
        sg = jax.nn.sigmoid(z1)
        hid = z1 * sg
        g = jax.nn.sigmoid(jnp.sum(wu * hid, axis=0, keepdims=True))
        g_t = row_to_tiles(g)

        def out_step(h, carry):
            for q in range(NG):
                store(ob, h, q, load(xb, h, q) * g_t[q])
            return carry

        ring_steps(RING_STEPS[1])
        slab_loop(0, H, out_step, 0)
        ring_steps(RING_STEPS[2])
        assert not pending

        parked = range(n_cyc, n_chunks)
        for c in rd_go[:-1]:
            c.wait()
        for u in parked:
            to_ring(u).wait()
        for u in parked:
            from_ring(u).start()
        start_writes(out_route, groups[0])
        rd_go[-1].wait()

        def dg_step(h, acc):
            return tuple(acc[q] + fold(load(xb, h, q) * load(gb, h, q)) for q in range(NG))

        acc = slab_loop(0, early // 2, dg_step, zeros)
        start_writes(out_route, groups[1])
        acc = slab_loop(early // 2, early, dg_step, acc)
        start_writes(out_route, groups[2])
        for u in parked:
            from_ring(u).wait()
        acc = slab_loop(early, H, dg_step, acc)
        dz2 = acc_to_row(acc) * g * (1.0 - g)
        dh = jnp.sum(wu * dz2, axis=1, keepdims=True)
        dz1 = dh * (sg + hid * (1.0 - sg))
        gwd_v[...] = (dz1 * s).astype(BF16)
        gwu_v[...] = (hid * dz2).astype(BF16)
        wr_w = [copy(gwd_v, gwd_hbm, w_sems.at[0]), copy(gwu_v, gwu_hbm, w_sems.at[1])]
        for c in wr_w:
            c.start()
        ds_t = row_to_tiles(jnp.sum(wd * dz1, axis=0, keepdims=True) * inv_n)

        def gx_step(h, carry):
            for q in range(NG):
                store(xb, h, q, load(gb, h, q) * g_t[q] + ds_t[q])
            return carry

        start_writes(out_route, groups[3], 0, columns // 2)
        slab_loop(0, H // 2, gx_step, 0)
        start_writes(out_route, groups[3], columns // 2, columns)
        slab_loop(H // 2, H, gx_step, 0)
        for group in groups:
            start_writes(gx_route, group)
        for c in [*wr_w, copy(*out_route), copy(*gx_route)]:
            c.wait()

    def kernel(*refs):
        dma = pltpu.SemaphoreType.DMA
        pl.run_scoped(lambda *sems: body(*refs, *sems),
                      dma(()), dma(()), dma(()), dma(()), dma((2,)), dma((SLOTS,)))

    any_spec = pl.BlockSpec(memory_space=pl.ANY)
    big = jax.ShapeDtypeStruct((NB, BLOCK, LANES), BF16)
    small = jax.ShapeDtypeStruct((R, C), BF16)
    out, gx, gwd_t, gwu = pl.pallas_call(
        kernel,
        in_specs=[any_spec] * 4,
        out_specs=[any_spec] * 4,
        out_shape=[big, big, small, small],
        scratch_shapes=(
            [pltpu.VMEM((NB, BLOCK, LANES), BF16)] * 3
            + [pltpu.VMEM((R, C), BF16)] * 4
            + [pltpu.SMEM((SLOTS, max(sizes), LANES), BF16)]
        ),
        compiler_params=pltpu.CompilerParams(vmem_limit_bytes=112 * 1024 * 1024),
    )(to_view(x), w_down.T, w_up, to_view(grad_out))
    return from_view(out), from_view(gx), gwd_t.T, gwu
```
